```python
import jax
import jax.numpy as jnp

def _softmax(x, axis=-1):
    return jax.nn.softmax(x, axis=axis)

def _gelu(x):
    return jax.nn.gelu(x, approximate=True)

def _silu(x):
    return jax.nn.silu(x)

def _sigmoid(x):
    return jax.nn.sigmoid(x)

def _layernorm(x, axis=-1, eps=1e-05):
    m = jnp.mean(x, axis=axis, keepdims=True)
    v = jnp.var(x, axis=axis, keepdims=True)
    return (x - m) / jnp.sqrt(v + eps)

def _scatter_add(tgt, idx, src, axis=0):
    return tgt.at[idx].add(src)

def _segment_sum(src, seg, n):
    return jax.ops.segment_sum(src, seg, n)

class _Rng:

    def __init__(self, key):
        self._k = key

    def _next(self):
        self._k, sub = jax.random.split(self._k)
        return sub

    def normal(self, shape):
        return jax.random.normal(self._next(), shape, dtype=jnp.bfloat16)

    def randint(self, lo, hi, shape):
        return jax.random.randint(self._next(), shape, lo, hi, dtype=jnp.int32)

    def uniform(self, shape, lo=0.0, hi=1.0):
        return jax.random.uniform(self._next(), shape, jnp.bfloat16, lo, hi)

    def permutation(self, n):
        return jax.random.permutation(self._next(), n)
kernel_name = 'adaLN_cond__compressed_kv_cla__mixer_s_mlp__decode'

def setup_inputs():
    _rng = _Rng(jax.random.key(int.from_bytes(__import__("os").urandom(4), "little")))
    _w = lambda a: (lambda t: t.astype(jnp.bfloat16) if jnp.issubdtype(t.dtype, jnp.floating) else t)(jnp.asarray(a))

    def _A_setup():
        B, H, Sq, Sk, D, M = (8, 32, 1, 4096, 128, 512)
        Dc = 4 * D
        return {'x': _w((lambda *s: _rng.normal(s) * 0.05)(B, Sq, M)), 'c_kv': _w((lambda *s: _rng.normal(s) * 0.05)(B, Sk, Dc)), 'w_q': _w((lambda *s: _rng.normal(s) * 0.05)(M, H, D) * M ** (-0.5)), 'w_uk': _w((lambda *s: _rng.normal(s) * 0.05)(Dc, H, D) * Dc ** (-0.5)), 'w_uv': _w((lambda *s: _rng.normal(s) * 0.05)(Dc, H, D) * Dc ** (-0.5)), 'w_o': _w((lambda *s: _rng.normal(s) * 0.05)(H, D, M) * (H * D) ** (-0.5))}
    _A_in = _A_setup()

    def _B_setup():
        B, S, D, F = (8, 1, 512, 1792)
        return {'x': _w((lambda *s: _rng.normal(s) * 0.05)(B, S, D)), 'w1': _w((lambda *s: _rng.normal(s) * 0.05)(D, D) * D ** (-0.5)), 'w2': _w((lambda *s: _rng.normal(s) * 0.05)(D, D) * D ** (-0.5)), 'w3': _w((lambda *s: _rng.normal(s) * 0.05)(D, F) * D ** (-0.5)), 'w4': _w((lambda *s: _rng.normal(s) * 0.05)(F, D) * F ** (-0.5))}
    _B_in = _B_setup()
    return {'A_x': _A_in['x'], 'A_c_kv': _A_in['c_kv'], 'A_w_q': _A_in['w_q'], 'A_w_uk': _A_in['w_uk'], 'A_w_uv': _A_in['w_uv'], 'A_w_o': _A_in['w_o'], 'B_x': _B_in['x'], 'B_w1': _B_in['w1'], 'B_w2': _B_in['w2'], 'B_w3': _B_in['w3'], 'B_w4': _B_in['w4'], 'c': _w((lambda *s: _rng.normal(s) * 0.05)(8, 512)), 'w_mod': _w((lambda *s: _rng.normal(s) * 0.05)(512, 6 * 512) * 512 ** (-0.5))}

def reference(A_x, A_c_kv, A_w_q, A_w_uk, A_w_uv, A_w_o, B_x, B_w1, B_w2, B_w3, B_w4, c, w_mod):

    def _A_ref(x, c_kv, w_q, w_uk, w_uv, w_o):
        B, Sq, M = (x.shape[0], x.shape[1], x.shape[2])
        Sk = c_kv.shape[1]
        H, D = (w_q.shape[1], w_q.shape[2])
        q = jnp.einsum('bqm,mhd->bhqd', x, w_q)
        k = jnp.einsum('bkc,chd->bhkd', c_kv, w_uk)
        v = jnp.einsum('bkc,chd->bhkd', c_kv, w_uv)
        scores = jnp.einsum('bhqd,bhkd->bhqk', q, k) * D ** (-0.5)
        off = Sk - Sq
        qi = jnp.arange(Sq)[:, None]
        kj = jnp.arange(Sk)[None, :]
        cmask = kj <= qi + off
        scores = jnp.where(cmask[None, None], scores, -1000000000.0)
        p = _softmax(scores, axis=-1)
        ctx = jnp.einsum('bhqk,bhkd->bhqd', p, v)
        return jnp.einsum('bhqd,hdm->bqm', ctx, w_o)

    def _B_ref(x, w1, w2, w3, w4):
        B, S, D = x.shape
        h = _gelu(_layernorm(x, axis=-1) @ w1)
        c = D // 4
        g0 = jnp.pad(h[:, :, 0 * c:1 * c], ((0, 0), (1, 0), (0, 0)))[:, :S, :]
        g1 = jnp.pad(h[:, :, 1 * c:2 * c], ((0, 0), (0, 1), (0, 0)))[:, 1:, :]
        g2 = jnp.pad(h[:, :, 2 * c:3 * c], ((0, 0), (2, 0), (0, 0)))[:, :S, :]
        g3 = jnp.pad(h[:, :, 3 * c:], ((0, 0), (0, 2), (0, 0)))[:, 2:, :]
        hs = jnp.concatenate([g0, g1, g2, g3], axis=-1) @ w2
        x1 = x + hs
        h2 = _gelu(_layernorm(x1, axis=-1) @ w3) @ w4
        return x1 + h2
    x = A_x
    mod = (_silu(c) @ w_mod).reshape(c.shape[0], 6, 1, -1)
    sa, ca, ga, sb, cb, gb = (mod[:, 0].copy(), mod[:, 1].copy(), mod[:, 2].copy(), mod[:, 3].copy(), mod[:, 4].copy(), mod[:, 5].copy())
    h = _layernorm(x, axis=-1) * (1 + ca) + sa
    x = x + ga * _A_ref(h, A_c_kv, A_w_q, A_w_uk, A_w_uv, A_w_o)
    h = _layernorm(x, axis=-1) * (1 + cb) + sb
    x = x + gb * _B_ref(h, B_w1, B_w2, B_w3, B_w4)
    return x
```

```python
import jax
import jax.numpy as jnp
import jax.experimental.pallas as pl
import jax.experimental.pallas.tpu as pltpu

F32 = jnp.float32
BF16 = jnp.bfloat16
U32 = jnp.uint32
_NT = (((1,), (1,)), ((), ()))
_LANES = 128


def _layernorm(x, eps=1e-05):
    m = jnp.mean(x, axis=-1, keepdims=True)
    d = x - m
    v = jnp.mean(d * d, axis=-1, keepdims=True)
    return d * jax.lax.rsqrt(v + eps)


def _dot(a, b):
    return jnp.dot(a, b, preferred_element_type=F32)


def _head_pair(w32_ref, i, rows, pairs):
    u = w32_ref[pl.ds(i, rows, stride=pairs), :]
    lo = pltpu.bitcast(u << 16, F32).astype(BF16)
    hi = pltpu.bitcast(u & jnp.uint32(0xFFFF0000), F32).astype(BF16)
    return lo, hi


def _kernel(
    x_hbm, ckv_hbm, wq_hbm, wuk_hbm, wuv_hbm, wo_hbm, w3_hbm, w4_hbm, c_hbm, wmod_hbm,
    out_ref,
    x_v, c_v, wmod_v, wq_v, wuk_v, ckv_v, wuv_v, wo_v, w3_v, w4_v,
    qa_v, o_v, ctx_v, sems,
    *, B, H, D, M, Dc, Sk, Fd, w4_splits,
):
    pairs = H // 2
    ct = Dc // _LANES

    copies = []

    def enqueue(src, dst):
        cp = pltpu.make_async_copy(src, dst, sems.at[len(copies)])
        cp.start()
        copies.append(cp)
        return cp

    cp_wmod = enqueue(wmod_hbm, wmod_v)
    cp_c = enqueue(c_hbm, c_v)
    cp_x = enqueue(x_hbm, x_v)
    cp_wq = enqueue(wq_hbm.bitcast(U32), wq_v)
    cp_wuk = enqueue(wuk_hbm.bitcast(U32), wuk_v)
    ckv_sem0 = len(copies)
    for b in range(B):
        enqueue(ckv_hbm.at[b], ckv_v.at[b])
    cp_wuv = enqueue(wuv_hbm.bitcast(U32), wuv_v)
    cp_wo = enqueue(wo_hbm, wo_v)
    cp_w3 = enqueue(w3_hbm, w3_v)
    cp_w4 = [
        enqueue(w4_hbm.at[pl.ds(lo, hi - lo)], w4_v.at[pl.ds(lo, hi - lo)])
        for lo, hi in zip(w4_splits[:-1], w4_splits[1:])
    ]

    cp_c.wait()
    cv = c_v[...].astype(F32)
    sc = (cv * jax.nn.sigmoid(cv)).astype(BF16)
    cp_x.wait()
    x = x_v[...].astype(F32)
    ln_x = _layernorm(x)
    cp_wmod.wait()
    mod = _dot(sc, wmod_v[...])
    sa, ca, ga, sb, cb, gb = (mod[:, i * M:(i + 1) * M] for i in range(6))
    h = (ln_x * (1.0 + ca) + sa).astype(BF16)

    cp_wq.wait()
    wq32 = wq_v

    def q_body(i, carry):
        lo, hi = _head_pair(wq32, i, M, pairs)
        ctx_v[2 * i] = _dot(h, lo)
        ctx_v[2 * i + 1] = _dot(h, hi)
        return carry

    jax.lax.fori_loop(0, pairs, q_body, 0)

    cp_wuk.wait()
    wuk32 = wuk_v
    scale = D ** (-0.5)

    def qa_body(i, carry):
        for j, w in enumerate(_head_pair(wuk32, i, Dc, pairs)):
            hd = 2 * i + j
            qa = jax.lax.dot_general(
                ctx_v[hd].astype(BF16), w, _NT, preferred_element_type=F32) * scale
            row = pl.multiple_of(hd * B, B)
            for t in range(ct):
                qa_v[t, pl.ds(row, B), :] = qa[:, t * _LANES:(t + 1) * _LANES]
        return carry

    jax.lax.fori_loop(0, pairs, qa_body, 0)

    def attn_body(b, carry):
        pltpu.make_async_copy(ckv_hbm.at[b], ckv_v.at[b], sems.at[ckv_sem0 + b]).wait()
        qa = jnp.concatenate(
            [qa_v[t, pl.ds(b, H, stride=B), :] for t in range(ct)], axis=1
        ).astype(BF16)
        s = jax.lax.dot_general(qa, ckv_v[b], _NT, preferred_element_type=F32)
        m = jnp.max(s, axis=-1, keepdims=True)
        p = jnp.exp(s - m)
        l = jnp.sum(p, axis=-1, keepdims=True)
        o = _dot(p.astype(BF16), ckv_v[b]) * (1.0 / l)
        for t in range(ct):
            o_v[t, pl.ds(b, H, stride=B), :] = o[:, t * _LANES:(t + 1) * _LANES]
        return carry

    jax.lax.fori_loop(0, B, attn_body, 0)

    cp_wuv.wait()
    wuv32 = wuv_v

    def ctx_body(i, carry):
        for j, w in enumerate(_head_pair(wuv32, i, Dc, pairs)):
            hd = 2 * i + j
            row = pl.multiple_of(hd * B, B)
            o = jnp.concatenate(
                [o_v[t, pl.ds(row, B), :] for t in range(ct)], axis=1).astype(BF16)
            ctx_v[hd] = _dot(o, w)
        return carry

    jax.lax.fori_loop(0, pairs, ctx_body, 0)

    cp_wo.wait()
    ctx = jnp.concatenate([ctx_v[hd] for hd in range(H)], axis=1).astype(BF16)
    attn = _dot(ctx, wo_v[...])
    x1 = x + ga * attn
    hb = _layernorm(x1) * (1.0 + cb) + sb
    ln_hb = _layernorm(hb).astype(BF16)

    cp_w3.wait()
    g = jax.nn.gelu(_dot(ln_hb, w3_v[...]), approximate=True).astype(BF16)
    y = hb
    for cp, lo, hi in zip(cp_w4, w4_splits[:-1], w4_splits[1:]):
        cp.wait()
        y = y + _dot(g[:, lo:hi], w4_v[lo:hi, :])
    out = x1 + gb * y
    out_ref[...] = out.astype(out_ref.dtype)


@jax.jit
def pallas_adaLN_cond__compressed_kv_cla__mixer_s_mlp__decode_kernel(
    A_x: jax.Array,
    A_c_kv: jax.Array,
    A_w_q: jax.Array,
    A_w_uk: jax.Array,
    A_w_uv: jax.Array,
    A_w_o: jax.Array,
    B_x: jax.Array,
    B_w1: jax.Array,
    B_w2: jax.Array,
    B_w3: jax.Array,
    B_w4: jax.Array,
    c: jax.Array,
    w_mod: jax.Array,
):
    del B_x, B_w1, B_w2
    B, Sq, M = A_x.shape
    _, Sk, Dc = A_c_kv.shape
    _, H, D = A_w_q.shape
    Fd = B_w3.shape[1]
    assert Sq == 1 and D == _LANES and H % 2 == 0 and Dc % _LANES == 0 and B == 8

    w4_splits = (0, 768, 1280, 1536, 1664, Fd)
    n_copies = 8 + B + len(w4_splits) - 1

    def kernel(*refs):
        _kernel(*refs, B=B, H=H, D=D, M=M, Dc=Dc, Sk=Sk, Fd=Fd, w4_splits=w4_splits)

    hbm = pl.BlockSpec(memory_space=pl.ANY)
    out = pl.pallas_call(
        kernel,
        in_specs=[hbm] * 10,
        out_specs=pl.BlockSpec(memory_space=pltpu.VMEM),
        out_shape=jax.ShapeDtypeStruct((B, M), A_x.dtype),
        scratch_shapes=[
            pltpu.VMEM((B, M), BF16),
            pltpu.VMEM((B, M), BF16),
            pltpu.VMEM((M, 6 * M), BF16),
            pltpu.VMEM((M * H // 2, D), U32),
            pltpu.VMEM((Dc * H // 2, D), U32),
            pltpu.VMEM((B, Sk, Dc), BF16),
            pltpu.VMEM((Dc * H // 2, D), U32),
            pltpu.VMEM((H * D, M), BF16),
            pltpu.VMEM((M, Fd), BF16),
            pltpu.VMEM((Fd, M), BF16),
            pltpu.VMEM((Dc // _LANES, H * B, _LANES), F32),
            pltpu.VMEM((Dc // _LANES, H * B, _LANES), F32),
            pltpu.VMEM((H, B, D), F32),
            pltpu.SemaphoreType.DMA((n_copies,)),
        ],
        compiler_params=pltpu.CompilerParams(
            vmem_limit_bytes=96 * 2**20, disable_semaphore_checks=True),
    )(
        A_x.reshape(B, M),
        A_c_kv,
        A_w_q.reshape(M * H, D),
        A_w_uk.reshape(Dc * H, D),
        A_w_uv.reshape(Dc * H, D),
        A_w_o.reshape(H * D, M),
        B_w3,
        B_w4,
        c,
        w_mod,
    )
    return out.reshape(B, Sq, M)
```

```python
import functools

import jax
import jax.numpy as jnp
import jax.experimental.pallas as pl
import jax.experimental.pallas.tpu as pltpu

F32 = jnp.float32
BF16 = jnp.bfloat16
U32 = jnp.uint32
LANES = 128
SUBLANES = 8


def _layernorm(x, eps=1e-05):
    d = x - jnp.mean(x, axis=-1, keepdims=True)
    v = jnp.mean(d * d, axis=-1, keepdims=True)
    return d * jax.lax.rsqrt(v + eps)


def _dot(a, b):
    return jnp.dot(a, b, preferred_element_type=F32)


def _dot_nt(a, b):
    return jax.lax.dot_general(
        a, b, (((1,), (1,)), ((), ())), preferred_element_type=F32)


def _store_as_words(w_ref, words_ref, step=1024):
    step = min(step, w_ref.shape[0])
    assert w_ref.shape[0] % step == 0

    def body(i, carry):
        src = pl.ds(pl.multiple_of(i * step, step), step)
        dst = pl.ds(pl.multiple_of(i * (step // 2), step // 2), step // 2)
        words_ref[dst, :] = pltpu.bitcast(w_ref[src, :], U32)
        return carry

    jax.lax.fori_loop(0, w_ref.shape[0] // step, body, 0)


def _head_pair(words_ref, i, rows, pairs):
    u = words_ref[pl.ds(i, rows, stride=pairs), :]
    even = pltpu.bitcast(u << 16, F32).astype(BF16)
    odd = pltpu.bitcast(u & jnp.uint32(0xFFFF0000), F32).astype(BF16)
    return even, odd


def _kernel(
    x_hbm, ckv_hbm, wq_hbm, wuk_hbm, wuv_hbm, wo_hbm, w3_hbm, w4_hbm, c_hbm, wmod_hbm,
    out_ref,
    x_v, ckv_v, wq_v, wuk_v, wuv_v, wo_v, w3_v, w4_v, c_v, wmod_v,
    words_v, qa_v, lat_v, head_v, sems,
    *, w4_chunks,
):
    B, M = x_v.shape
    Dc = ckv_v.shape[-1]
    H, _, D = head_v.shape
    pairs = H // 2
    lane_tiles = [slice(t, t + LANES) for t in range(0, Dc, LANES)]

    copies = []

    def enqueue(src, dst):
        cp = pltpu.make_async_copy(src, dst, sems.at[len(copies)])
        cp.start()
        copies.append(cp)
        return cp

    cp_wmod = enqueue(wmod_hbm, wmod_v)
    cp_c = enqueue(c_hbm, c_v)
    cp_x = enqueue(x_hbm, x_v)
    cp_wq = enqueue(wq_hbm, wq_v)
    cp_wuk = enqueue(wuk_hbm, wuk_v)
    ckv_sem = len(copies)
    for b in range(B):
        enqueue(ckv_hbm.at[b], ckv_v.at[b])
    cp_wuv = enqueue(wuv_hbm, wuv_v)
    cp_wo = enqueue(wo_hbm, wo_v)
    cp_w3 = enqueue(w3_hbm, w3_v)
    cp_w4 = [
        enqueue(w4_hbm.at[pl.ds(lo, hi - lo)], w4_v.at[pl.ds(lo, hi - lo)])
        for lo, hi in w4_chunks
    ]

    cp_wmod.wait()
    cp_c.wait()
    cp_x.wait()
    c = c_v[...].astype(F32)
    mod = _dot((c * jax.nn.sigmoid(c)).astype(BF16), wmod_v[...])
    sa, ca, ga, sb, cb, gb = (mod[:, i * M:(i + 1) * M] for i in range(6))
    x = x_v[...].astype(F32)
    h = (_layernorm(x) * (1.0 + ca) + sa).astype(BF16)

    cp_wq.wait()
    _store_as_words(wq_v, words_v)

    def q_body(i, carry):
        for j, w in enumerate(_head_pair(words_v, i, M, pairs)):
            head_v[2 * i + j] = _dot(h, w)
        return carry

    jax.lax.fori_loop(0, pairs, q_body, 0)

    cp_wuk.wait()
    _store_as_words(wuk_v, words_v)

    def qa_body(i, carry):
        for j, w in enumerate(_head_pair(words_v, i, Dc, pairs)):
            head = 2 * i + j
            qa = _dot_nt(head_v[head].astype(BF16), w) * D ** (-0.5)
            rows = pl.ds(pl.multiple_of(head * B, B), B)
            for t, cols in enumerate(lane_tiles):
                qa_v[t, rows, :] = qa[:, cols]
        return carry

    jax.lax.fori_loop(0, pairs, qa_body, 0)

    def attn_body(b, carry):
        pltpu.make_async_copy(ckv_hbm.at[b], ckv_v.at[b], sems.at[ckv_sem + b]).wait()
        rows = pl.ds(b, H, stride=B)
        qa = jnp.concatenate(
            [qa_v[t, rows, :] for t in range(len(lane_tiles))], axis=1)
        s = _dot_nt(qa.astype(BF16), ckv_v[b])
        p = jnp.exp(s - jnp.max(s, axis=-1, keepdims=True))
        denom = jnp.sum(p, axis=-1, keepdims=True)
        lat = _dot(p.astype(BF16), ckv_v[b]) * (1.0 / denom)
        for t, cols in enumerate(lane_tiles):
            lat_v[t, rows, :] = lat[:, cols]
        return carry

    jax.lax.fori_loop(0, B, attn_body, 0)

    cp_wuv.wait()
    _store_as_words(wuv_v, words_v)

    def ctx_body(i, carry):
        for j, w in enumerate(_head_pair(words_v, i, Dc, pairs)):
            head = 2 * i + j
            rows = pl.ds(pl.multiple_of(head * B, B), B)
            lat = jnp.concatenate(
                [lat_v[t, rows, :] for t in range(len(lane_tiles))], axis=1)
            head_v[head] = _dot(lat.astype(BF16), w)
        return carry

    jax.lax.fori_loop(0, pairs, ctx_body, 0)

    cp_wo.wait()
    ctx = jnp.concatenate([head_v[head] for head in range(H)], axis=1)
    x = x + ga * _dot(ctx.astype(BF16), wo_v[...])
    h = _layernorm(x) * (1.0 + cb) + sb
    h_norm = _layernorm(h).astype(BF16)

    cp_w3.wait()
    g = jax.nn.gelu(_dot(h_norm, w3_v[...]), approximate=True).astype(BF16)
    for cp, (lo, hi) in zip(cp_w4, w4_chunks):
        cp.wait()
        h = h + _dot(g[:, lo:hi], w4_v[lo:hi, :])
    out_ref[...] = (x + gb * h).astype(out_ref.dtype)


@jax.jit
def pallas_adaLN_cond__compressed_kv_cla__mixer_s_mlp__decode_kernel(
    A_x: jax.Array,
    A_c_kv: jax.Array,
    A_w_q: jax.Array,
    A_w_uk: jax.Array,
    A_w_uv: jax.Array,
    A_w_o: jax.Array,
    B_x: jax.Array,
    B_w1: jax.Array,
    B_w2: jax.Array,
    B_w3: jax.Array,
    B_w4: jax.Array,
    c: jax.Array,
    w_mod: jax.Array,
):
    del B_x, B_w1, B_w2
    B, Sq, M = A_x.shape
    _, Sk, Dc = A_c_kv.shape
    _, H, D = A_w_q.shape
    F = B_w3.shape[1]
    assert Sq == 1 and B == SUBLANES and D == LANES
    assert H % 2 == 0 and Dc % LANES == 0 and F % LANES == 0

    cuts = sorted({0, F} | {F - (LANES << k) for k in range(4) if F > (LANES << k)})
    w4_chunks = tuple(zip(cuts[:-1], cuts[1:]))

    words = pltpu.VMEM(((max(M, Dc) + 1) * H // 2, D), U32)
    head_major = pltpu.VMEM((Dc // LANES, H * B + B, LANES), F32)

    out = pl.pallas_call(
        functools.partial(_kernel, w4_chunks=w4_chunks),
        in_specs=[pl.BlockSpec(memory_space=pl.ANY)] * 10,
        out_specs=pl.BlockSpec(memory_space=pltpu.VMEM),
        out_shape=jax.ShapeDtypeStruct((B, M), A_x.dtype),
        scratch_shapes=[
            pltpu.VMEM((B, M), BF16),
            pltpu.VMEM((B, Sk, Dc), BF16),
            pltpu.VMEM((M * H, D), BF16),
            pltpu.VMEM((Dc * H, D), BF16),
            pltpu.VMEM((Dc * H, D), BF16),
            pltpu.VMEM((H * D, M), BF16),
            pltpu.VMEM((M, F), BF16),
            pltpu.VMEM((F, M), BF16),
            pltpu.VMEM(c.shape, BF16),
            pltpu.VMEM(w_mod.shape, BF16),
            words,
            head_major,
            head_major,
            pltpu.VMEM((H, B, D), F32),
            pltpu.SemaphoreType.DMA((8 + B + len(w4_chunks),)),
        ],
        compiler_params=pltpu.CompilerParams(
            vmem_limit_bytes=96 * 2**20,
            disable_semaphore_checks=True,
        ),
    )(
        A_x.reshape(B, M),
        A_c_kv,
        A_w_q.reshape(M * H, D),
        A_w_uk.reshape(Dc * H, D),
        A_w_uv.reshape(Dc * H, D),
        A_w_o.reshape(H * D, M),
        B_w3,
        B_w4,
        c,
        w_mod,
    )
    return out.reshape(B, Sq, M)
```

```python
import functools

import jax
import jax.numpy as jnp
import jax.experimental.pallas as pl
import jax.experimental.pallas.tpu as pltpu

F32 = jnp.float32
BF16 = jnp.bfloat16
U32 = jnp.uint32
LANES = 128
SUBLANES = 8


def _layernorm(x, eps=1e-05):
    d = x - jnp.mean(x, axis=-1, keepdims=True)
    v = jnp.mean(d * d, axis=-1, keepdims=True)
    return d * jax.lax.rsqrt(v + eps)


def _dot(a, b):
    return jnp.dot(a, b, preferred_element_type=F32)


def _dot_nt(a, b):
    return jax.lax.dot_general(
        a, b, (((1,), (1,)), ((), ())), preferred_element_type=F32)


def _store_as_words(w_ref, words_ref, step=1024):
    step = min(step, w_ref.shape[0])
    assert w_ref.shape[0] % step == 0

    def body(i, carry):
        src = pl.ds(pl.multiple_of(i * step, step), step)
        dst = pl.ds(pl.multiple_of(i * (step // 2), step // 2), step // 2)
        words_ref[dst, :] = pltpu.bitcast(w_ref[src, :], U32)
        return carry

    jax.lax.fori_loop(0, w_ref.shape[0] // step, body, 0)


def _head_pair(words_ref, i, rows, pairs):
    u = words_ref[pl.ds(i, rows, stride=pairs), :]
    even = pltpu.bitcast(u << 16, F32).astype(BF16)
    odd = pltpu.bitcast(u & jnp.uint32(0xFFFF0000), F32).astype(BF16)
    return even, odd


def _kernel(*refs, n_copies, w4_chunks):
    pl.run_scoped(
        functools.partial(_decode_step, *refs, w4_chunks=w4_chunks),
        pltpu.SemaphoreType.DMA((n_copies,)),
    )


def _decode_step(
    x_hbm, ckv_hbm, wq_hbm, wuk_hbm, wuv_hbm, wo_hbm, w3_hbm, w4_hbm, c_hbm, wmod_hbm,
    out_ref,
    x_v, ckv_v, wq_v, wuk_v, wuv_v, wo_v, w3_v, w4_v, c_v, wmod_v,
    words_v, qa_v, lat_v, head_v, sems,
    *, w4_chunks,
):
    B, M = x_v.shape
    Dc = ckv_v.shape[-1]
    H, _, D = head_v.shape
    pairs = H // 2
    lane_tiles = [slice(t, t + LANES) for t in range(0, Dc, LANES)]

    copies = []

    def enqueue(src, dst):
        cp = pltpu.make_async_copy(src, dst, sems.at[len(copies)])
        cp.start()
        copies.append(cp)
        return cp

    cp_wmod = enqueue(wmod_hbm, wmod_v)
    cp_c = enqueue(c_hbm, c_v)
    cp_x = enqueue(x_hbm, x_v)
    cp_wq = enqueue(wq_hbm, wq_v)
    cp_wuk = enqueue(wuk_hbm, wuk_v)
    ckv_sem = len(copies)
    for b in range(B):
        enqueue(ckv_hbm.at[b], ckv_v.at[b])
    cp_wuv = enqueue(wuv_hbm, wuv_v)
    cp_wo = enqueue(wo_hbm, wo_v)
    cp_w3 = enqueue(w3_hbm, w3_v)
    cp_w4 = [
        enqueue(w4_hbm.at[pl.ds(lo, hi - lo)], w4_v.at[pl.ds(lo, hi - lo)])
        for lo, hi in w4_chunks
    ]

    cp_wmod.wait()
    cp_c.wait()
    cp_x.wait()
    c = c_v[...].astype(F32)
    mod = _dot((c * jax.nn.sigmoid(c)).astype(BF16), wmod_v[...])
    sa, ca, ga, sb, cb, gb = (mod[:, i * M:(i + 1) * M] for i in range(6))
    x = x_v[...].astype(F32)
    h = (_layernorm(x) * (1.0 + ca) + sa).astype(BF16)

    cp_wq.wait()
    _store_as_words(wq_v, words_v)

    def q_body(i, carry):
        for j, w in enumerate(_head_pair(words_v, i, M, pairs)):
            head_v[2 * i + j] = _dot(h, w)
        return carry

    jax.lax.fori_loop(0, pairs, q_body, 0)

    cp_wuk.wait()
    _store_as_words(wuk_v, words_v)

    def qa_body(i, carry):
        for j, w in enumerate(_head_pair(words_v, i, Dc, pairs)):
            head = 2 * i + j
            qa = _dot_nt(head_v[head].astype(BF16), w) * D ** (-0.5)
            rows = pl.ds(pl.multiple_of(head * B, B), B)
            for t, cols in enumerate(lane_tiles):
                qa_v[t, rows, :] = qa[:, cols]
        return carry

    jax.lax.fori_loop(0, pairs, qa_body, 0)

    def attn_body(b, carry):
        pltpu.make_async_copy(ckv_hbm.at[b], ckv_v.at[b], sems.at[ckv_sem + b]).wait()
        rows = pl.ds(b, H, stride=B)
        qa = jnp.concatenate(
            [qa_v[t, rows, :] for t in range(len(lane_tiles))], axis=1)
        s = _dot_nt(qa.astype(BF16), ckv_v[b])
        p = jnp.exp(s - jnp.max(s, axis=-1, keepdims=True))
        denom = jnp.sum(p, axis=-1, keepdims=True)
        lat = _dot(p.astype(BF16), ckv_v[b]) * (1.0 / denom)
        for t, cols in enumerate(lane_tiles):
            lat_v[t, rows, :] = lat[:, cols]
        return carry

    jax.lax.fori_loop(0, B, attn_body, 0)

    cp_wuv.wait()
    _store_as_words(wuv_v, words_v)

    def ctx_body(i, carry):
        for j, w in enumerate(_head_pair(words_v, i, Dc, pairs)):
            head = 2 * i + j
            rows = pl.ds(pl.multiple_of(head * B, B), B)
            lat = jnp.concatenate(
                [lat_v[t, rows, :] for t in range(len(lane_tiles))], axis=1)
            head_v[head] = _dot(lat.astype(BF16), w)
        return carry

    jax.lax.fori_loop(0, pairs, ctx_body, 0)

    cp_wo.wait()
    ctx = jnp.concatenate([head_v[head] for head in range(H)], axis=1)
    x = x + ga * _dot(ctx.astype(BF16), wo_v[...])
    h = _layernorm(x) * (1.0 + cb) + sb
    h_norm = _layernorm(h).astype(BF16)

    cp_w3.wait()
    g = jax.nn.gelu(_dot(h_norm, w3_v[...]), approximate=True).astype(BF16)
    for cp, (lo, hi) in zip(cp_w4, w4_chunks):
        cp.wait()
        h = h + _dot(g[:, lo:hi], w4_v[lo:hi, :])
    out_ref[...] = (x + gb * h).astype(out_ref.dtype)


@jax.jit
def pallas_adaLN_cond__compressed_kv_cla__mixer_s_mlp__decode_kernel(
    A_x: jax.Array,
    A_c_kv: jax.Array,
    A_w_q: jax.Array,
    A_w_uk: jax.Array,
    A_w_uv: jax.Array,
    A_w_o: jax.Array,
    B_x: jax.Array,
    B_w1: jax.Array,
    B_w2: jax.Array,
    B_w3: jax.Array,
    B_w4: jax.Array,
    c: jax.Array,
    w_mod: jax.Array,
):
    del B_x, B_w1, B_w2
    B, Sq, M = A_x.shape
    _, Sk, Dc = A_c_kv.shape
    _, H, D = A_w_q.shape
    F = B_w3.shape[1]
    assert Sq == 1 and B == SUBLANES and D == LANES
    assert H % 2 == 0 and Dc % LANES == 0 and F % LANES == 0

    cuts = sorted({0, F} | {F - (LANES << k) for k in range(4) if F > (LANES << k)})
    w4_chunks = tuple(zip(cuts[:-1], cuts[1:]))

    words = pltpu.VMEM(((max(M, Dc) + 1) * H // 2, D), U32)
    head_major = pltpu.VMEM((Dc // LANES, H * B + B, LANES), F32)

    out = pl.pallas_call(
        functools.partial(_kernel, n_copies=8 + B + len(w4_chunks), w4_chunks=w4_chunks),
        in_specs=[pl.BlockSpec(memory_space=pl.ANY)] * 10,
        out_specs=pl.BlockSpec(memory_space=pltpu.VMEM),
        out_shape=jax.ShapeDtypeStruct((B, M), A_x.dtype),
        scratch_shapes=[
            pltpu.VMEM((B, M), BF16),
            pltpu.VMEM((B, Sk, Dc), BF16),
            pltpu.VMEM((M * H, D), BF16),
            pltpu.VMEM((Dc * H, D), BF16),
            pltpu.VMEM((Dc * H, D), BF16),
            pltpu.VMEM((H * D, M), BF16),
            pltpu.VMEM((M, F), BF16),
            pltpu.VMEM((F, M), BF16),
            pltpu.VMEM(c.shape, BF16),
            pltpu.VMEM(w_mod.shape, BF16),
            words,
            head_major,
            head_major,
            pltpu.VMEM((H, B, D), F32),
        ],
        compiler_params=pltpu.CompilerParams(vmem_limit_bytes=96 * 2**20),
    )(
        A_x.reshape(B, M),
        A_c_kv,
        A_w_q.reshape(M * H, D),
        A_w_uk.reshape(Dc * H, D),
        A_w_uv.reshape(Dc * H, D),
        A_w_o.reshape(H * D, M),
        B_w3,
        B_w4,
        c,
        w_mod,
    )
    return out.reshape(B, Sq, M)
```
